```python
import jax
import jax.numpy as jnp

def _softmax(x, axis=-1):
    return jax.nn.softmax(x, axis=axis)
def _gelu(x):
    return jax.nn.gelu(x, approximate=True)
def _silu(x):
    return jax.nn.silu(x)
def _sigmoid(x):
    return jax.nn.sigmoid(x)
def _layernorm(x, axis=-1, eps=1e-5):
    m = jnp.mean(x, axis=axis, keepdims=True)
    v = jnp.var(x, axis=axis, keepdims=True)
    return (x - m) / jnp.sqrt(v + eps)
def _scatter_add(tgt, idx, src, axis=0):
    return tgt.at[idx].add(src)
def _segment_sum(src, seg, n):
    return jax.ops.segment_sum(src, seg, n)
class _Rng:
    def __init__(self, key):
        self._k = key
    def _next(self):
        self._k, sub = jax.random.split(self._k)
        return sub
    def normal(self, shape):
        return jax.random.normal(self._next(), shape, dtype=jnp.bfloat16)
    def randint(self, lo, hi, shape):
        return jax.random.randint(self._next(), shape, lo, hi, dtype=jnp.int32)
    def uniform(self, shape, lo=0.0, hi=1.0):
        return jax.random.uniform(self._next(), shape, jnp.bfloat16, lo, hi)
    def permutation(self, n):
        return jax.random.permutation(self._next(), n)


kernel_name = 'sequential_preLN__sliding_block_cached__moe_arch_mod__decode'

def setup_inputs():
    _rng = _Rng(jax.random.key(int.from_bytes(__import__("os").urandom(4), "little")))
    _w = (lambda a: (lambda t: t.astype(jnp.bfloat16) if jnp.issubdtype(t.dtype, jnp.floating) else t)(jnp.asarray(a)))
    def _A_setup():
        B, Sq, D = 1, 1, 640
        Hq, Hkv, Sk, Dh = 32, 32, 32768, 192
        assert Hq % Hkv == 0, (Hq, Hkv)
        return {
            "x": _w((lambda *s: _rng.normal(s) * 0.05)(B, Sq, D)),
            "k_cache": _w((lambda *s: _rng.normal(s) * 0.05)(B, Hkv, Sk, Dh)),
            "v_cache": _w((lambda *s: _rng.normal(s) * 0.05)(B, Hkv, Sk, Dh)),
            "wq": _w((lambda *s: _rng.normal(s) * 0.05)(D, Hq * Dh) * (D ** -0.5)),
            "wo": _w((lambda *s: _rng.normal(s) * 0.05)(Hq * Dh, D) * ((Hq * Dh) ** -0.5)),
        }
    _A_in = _A_setup()

    def _B_setup():
        B, S, D, F, C = 1, 1, 640, 1536, 1
        return {
            "x": _w((lambda *s: _rng.normal(s) * 0.05)(B, S, D)),
            "w_r": _w((lambda *s: _rng.normal(s) * 0.05)(D)),
            "w_gate": _w((lambda *s: _rng.normal(s) * 0.05)(D, F)),
            "w_up": _w((lambda *s: _rng.normal(s) * 0.05)(D, F)),
            "w_down": _w((lambda *s: _rng.normal(s) * 0.05)(F, D)),
        }
    _B_in = _B_setup()

    return {
        "A_x": _A_in["x"],
        "A_k_cache": _A_in["k_cache"],
        "A_v_cache": _A_in["v_cache"],
        "A_wq": _A_in["wq"],
        "A_wo": _A_in["wo"],
        "B_x": _B_in["x"],
        "B_w_r": _B_in["w_r"],
        "B_w_gate": _B_in["w_gate"],
        "B_w_up": _B_in["w_up"],
        "B_w_down": _B_in["w_down"],
    }

def reference(A_x, A_k_cache, A_v_cache, A_wq, A_wo, B_x, B_w_r, B_w_gate, B_w_up, B_w_down):
    def _A_ref(x, k_cache, v_cache, wq, wo):
        B, Sq, D = x.shape
        Hq, Dh = 32, 192
        Hkv, Sk = k_cache.shape[1], k_cache.shape[2]
        W = min(4096, max(256, Sk // 4))
        rep = Hq // Hkv
        q = (lambda x, *d: x.transpose(*d))((x @ wq).reshape(B, Sq, Hq, Dh), 0, 2, 1, 3)
        k = jnp.repeat(k_cache[:, :, Sk - W:, :], rep, axis=1)
        v = jnp.repeat(v_cache[:, :, Sk - W:, :], rep, axis=1)
        scores = jnp.einsum("bhqd,bhkd->bhqk", q, k) * (Dh ** -0.5)
        p = _softmax(scores, axis=-1)
        o = jnp.einsum("bhqk,bhkd->bhqd", p, v)
        return (lambda x, *d: x.transpose(*d))(o, 0, 2, 1, 3).reshape(B, Sq, Hq * Dh) @ wo

    def _B_ref(x, w_r, w_gate, w_up, w_down):
        B, S, D = x.shape
        C = 1
        r = x @ w_r
        idx = jnp.argsort(-r, axis=-1)[:, :C]
        idx_e = jnp.repeat(idx.reshape(B, C, 1), D, axis=2)
        x_sel = jnp.take_along_axis(x, idx_e, axis=1)
        g = _silu(x_sel @ w_gate)
        u = x_sel @ w_up
        y = (g * u) @ w_down
        r_sel = _sigmoid(jnp.take_along_axis(r, idx, axis=1))
        y = y * r_sel.reshape(B, C, 1)
        b_off = (jnp.arange(B) * S).reshape(B, 1)
        flat_idx = (idx + b_off).reshape(B * C)
        zero = (x * 0.0).reshape(B * S, D)
        upd = _scatter_add(zero, flat_idx, y.reshape(B * C, D), axis=0)
        return x + upd.reshape(B, S, D)

    x = A_x
    h = x + _A_ref(_layernorm(x, axis=-1), A_k_cache, A_v_cache, A_wq, A_wo)
    h2 = h + _B_ref(_layernorm(h, axis=-1), B_w_r, B_w_gate, B_w_up, B_w_down)
    return h2
```

```python
import functools

import jax
import jax.numpy as jnp
import jax.experimental.pallas as pl
import jax.experimental.pallas.tpu as pltpu

_HQ, _DH = 32, 192
_G = 2
_NBUF = 3
_FC = 512


def _layernorm(x):
    m = jnp.mean(x, axis=-1, keepdims=True)
    c = x - m
    v = jnp.mean(c * c, axis=-1, keepdims=True)
    return c / jnp.sqrt(v + 1e-5)


def _dot(a, b):
    return jnp.dot(a, b, preferred_element_type=jnp.float32)


def _kernel(x_hbm, wr_hbm, k_hbm, v_hbm, wq_hbm, wo_hbm, wg_hbm, wu_hbm, wd_hbm,
            o_ref, kb, vb, wqb, wob, wgb, wub, wdb, x_ref, wr_ref, sem, fsem, xsem,
            *, g, nbuf, fc, w):
    rows = g * _DH
    sk = k_hbm.shape[1]
    nsteps = k_hbm.shape[0] // rows
    nf = wg_hbm.shape[1] // fc
    bf16 = jnp.bfloat16

    def copies(i, slot):
        r = pl.ds(pl.multiple_of(i * rows, rows), rows)
        win = pl.ds(sk - w, w)
        return (
            pltpu.make_async_copy(wq_hbm.at[:, r], wqb.at[slot], sem.at[0, slot]),
            pltpu.make_async_copy(k_hbm.at[r, win], kb.at[slot], sem.at[1, slot]),
            pltpu.make_async_copy(v_hbm.at[r, win], vb.at[slot], sem.at[2, slot]),
            pltpu.make_async_copy(wo_hbm.at[r, :], wob.at[slot], sem.at[3, slot]),
        )

    def ffn_copies(c):
        cs = pl.ds(c * fc, fc)
        return (
            pltpu.make_async_copy(wg_hbm.at[:, cs], wgb.at[c], fsem.at[0, c]),
            pltpu.make_async_copy(wu_hbm.at[:, cs], wub.at[c], fsem.at[1, c]),
            pltpu.make_async_copy(wd_hbm.at[cs, :], wdb.at[c], fsem.at[2, c]),
        )

    def start(cps):
        for cp in cps:
            cp.start()

    cx = pltpu.make_async_copy(x_hbm, x_ref, xsem.at[0])
    cr = pltpu.make_async_copy(wr_hbm, wr_ref, xsem.at[1])
    for i in range(nbuf - 1):
        start(copies(i, i))
        if i == 0:
            cx.start()
            cr.start()
    cx.wait()

    x = x_ref[0].astype(jnp.float32)
    xn = jnp.broadcast_to(_layernorm(x), (16, x.shape[1])).astype(bf16)

    row = jax.lax.broadcasted_iota(jnp.int32, (16, rows), 0)
    col = jax.lax.broadcasted_iota(jnp.int32, (16, rows), 1)
    diag = jnp.logical_and(col >= row * _DH, col < (row + 1) * _DH)

    def step(i, acc):
        slot = jax.lax.rem(i, nbuf)
        nxt = i + nbuf - 1

        @pl.when(nxt < nsteps)
        def _():
            start(copies(nxt, jax.lax.rem(nxt, nbuf)))

        @pl.when(nxt == nsteps)
        def _():
            for c in range(nf):
                start(ffn_copies(c))

        cq, ck, cv, co = copies(i, slot)
        cq.wait()
        q = _dot(xn, wqb[slot])
        qd = jnp.where(diag, q, 0.0).astype(bf16)
        ck.wait()
        s = _dot(qd, kb[slot]) * (_DH ** -0.5)
        m = jnp.max(s, axis=-1, keepdims=True)
        p = jnp.exp(s - m)
        l = jnp.sum(p, axis=-1, keepdims=True)
        cv.wait()
        o = jax.lax.dot_general(p.astype(bf16), vb[slot], (((1,), (1,)), ((), ())),
                                preferred_element_type=jnp.float32)
        o = jnp.where(diag, o / l, 0.0).astype(bf16)
        co.wait()
        return acc + _dot(o, wob[slot])

    acc = jax.lax.fori_loop(0, nsteps, step, jnp.zeros(xn.shape, jnp.float32))
    h = x + jnp.sum(acc, axis=0, keepdims=True)
    z = _layernorm(h)
    cr.wait()
    zr = z.astype(bf16).astype(jnp.float32)
    r = jnp.sum(zr * wr_ref[...].astype(jnp.float32).reshape(1, -1), axis=-1, keepdims=True)
    zb = jnp.broadcast_to(z, xn.shape).astype(bf16)
    y = jnp.zeros(xn.shape, jnp.float32)
    for c in range(nf):
        cg, cu, cd = ffn_copies(c)
        cg.wait()
        gate = _dot(zb, wgb[c])
        cu.wait()
        up = _dot(zb, wub[c])
        act = (gate * jax.nn.sigmoid(gate) * up).astype(bf16)
        cd.wait()
        y = y + _dot(act, wdb[c])
    upd = z * 0.0 + y[0:1] * jax.nn.sigmoid(r)
    o_ref[0] = (h + (z + upd)).astype(o_ref.dtype)


def _run(A_x, A_k_cache, A_v_cache, A_wq, A_wo, B_w_r, B_w_gate, B_w_up, B_w_down,
         g=_G, nbuf=_NBUF, fc=_FC):
    _, hkv, sk, dh = A_k_cache.shape
    d = A_x.shape[-1]
    f = B_w_gate.shape[1]
    w = min(4096, max(256, sk // 4))
    rows = g * dh
    kt = A_k_cache.transpose(0, 1, 3, 2).reshape(hkv * dh, sk)
    vt = A_v_cache.transpose(0, 1, 3, 2).reshape(hkv * dh, sk)
    bf16 = jnp.bfloat16
    vmem = pl.BlockSpec(memory_space=pltpu.VMEM)
    hbm = pl.BlockSpec(memory_space=pl.ANY)
    return pl.pallas_call(
        functools.partial(_kernel, g=g, nbuf=nbuf, fc=fc, w=w),
        out_shape=jax.ShapeDtypeStruct(A_x.shape, A_x.dtype),
        in_specs=[hbm] * 9,
        out_specs=vmem,
        scratch_shapes=[
            pltpu.VMEM((nbuf, rows, w), bf16),
            pltpu.VMEM((nbuf, rows, w), bf16),
            pltpu.VMEM((nbuf, d, rows), bf16),
            pltpu.VMEM((nbuf, rows, d), bf16),
            pltpu.VMEM((f // fc, d, fc), bf16),
            pltpu.VMEM((f // fc, d, fc), bf16),
            pltpu.VMEM((f // fc, fc, d), bf16),
            pltpu.VMEM(A_x.shape, bf16),
            pltpu.VMEM(B_w_r.shape, bf16),
            pltpu.SemaphoreType.DMA((4, nbuf)),
            pltpu.SemaphoreType.DMA((3, f // fc)),
            pltpu.SemaphoreType.DMA((2,)),
        ],
        compiler_params=pltpu.CompilerParams(vmem_limit_bytes=100 * 2 ** 20),
    )(A_x, B_w_r, kt, vt, A_wq, A_wo, B_w_gate, B_w_up, B_w_down)


@jax.jit
def pallas_sequential_preLN__sliding_block_cached__moe_arch_mod__decode_kernel(
    A_x: jax.Array,
    A_k_cache: jax.Array,
    A_v_cache: jax.Array,
    A_wq: jax.Array,
    A_wo: jax.Array,
    B_x: jax.Array,
    B_w_r: jax.Array,
    B_w_gate: jax.Array,
    B_w_up: jax.Array,
    B_w_down: jax.Array,
):
    return _run(A_x, A_k_cache, A_v_cache, A_wq, A_wo, B_w_r, B_w_gate, B_w_up, B_w_down)
```
